```python
import os as _os
_os.environ.setdefault("JAX_PLATFORMS", "cpu")
import jax
import jax.numpy as jnp

def _softmax(x, axis=-1):
    return jax.nn.softmax(x, axis=axis)
def _gelu(x):
    return jax.nn.gelu(x, approximate=True)
def _silu(x):
    return jax.nn.silu(x)
def _sigmoid(x):
    return jax.nn.sigmoid(x)
def _layernorm(x, axis=-1, eps=1e-5):
    m = jnp.mean(x, axis=axis, keepdims=True)
    v = jnp.var(x, axis=axis, keepdims=True)
    return (x - m) / jnp.sqrt(v + eps)
def _scatter_add(tgt, idx, src, axis=0):
    return tgt.at[idx].add(src)
def _segment_sum(src, seg, n):
    return jax.ops.segment_sum(src, seg, n)
class _Rng:
    def __init__(self, key):
        self._k = key
    def _next(self):
        self._k, sub = jax.random.split(self._k)
        return sub
    def normal(self, shape):
        return jax.random.normal(self._next(), shape, dtype=jnp.bfloat16)
    def randint(self, lo, hi, shape):
        return jax.random.randint(self._next(), shape, lo, hi, dtype=jnp.int32)
    def uniform(self, shape, lo=0.0, hi=1.0):
        return jax.random.uniform(self._next(), shape, jnp.bfloat16, lo, hi)
    def permutation(self, n):
        return jax.random.permutation(self._next(), n)


kernel_name = 'standalone__mha_softmax__near_ridge'

def setup_inputs():
    _rng = _Rng(jax.random.key(int.from_bytes(__import__("os").urandom(4), "little")))
    _w = (lambda a: (lambda t: t.astype(jnp.bfloat16) if jnp.issubdtype(t.dtype, jnp.floating) else t)(jnp.asarray(a)))
    B, H, Sq, Sk, D = 16, 16, 256, 256, 256
    return {
        "q": _w((lambda *s: _rng.normal(s) * 0.4)(B, H, Sq, D)),
        "k": _w((lambda *s: _rng.normal(s) * 0.4)(B, H, Sk, D)),
        "v": _w((lambda *s: _rng.normal(s) * 0.05)(B, H, Sk, D)),
    }

def reference(q, k, v):
    scale = q.shape[-1] ** -0.5
    scores = jnp.einsum("bhqd,bhkd->bhqk", q, k) * scale
    p = _softmax(scores, axis=-1)
    return jnp.einsum("bhqk,bhkd->bhqd", p, v)
```

```python
import math

import jax
import jax.numpy as jnp
import jax.experimental.pallas as pl
import jax.experimental.pallas.tpu as pltpu

GS = 8
LOOKAHEAD = 3
W_EARLY = 2


def _attention_head(q, k, v, c):
    s = jax.lax.dot_general(q, k, (((1,), (1,)), ((), ())),
                            preferred_element_type=jnp.float32)
    m = jnp.max(s, axis=-1, keepdims=True)
    e = jnp.exp2((s - m) * c)
    l = jnp.sum(e, axis=-1, keepdims=True)
    o = jnp.dot(e.astype(v.dtype), v, preferred_element_type=jnp.float32)
    return o * (1.0 / l)


@jax.jit
def pallas_standalone__mha_softmax__near_ridge_kernel(
    q: jax.Array,
    k: jax.Array,
    v: jax.Array,
):
    B, H, Sq, D = q.shape
    Sk = k.shape[2]
    NH = B * H
    gs = math.gcd(GS, NH)
    T = NH // gs
    la = min(LOOKAHEAD, T)
    nbuf = la + 1
    w_early = min(W_EARLY, T)
    c = (D ** -0.5) * math.log2(math.e)

    def kernel_function(q_hbm, k_hbm, v_hbm, o_hbm, qb, kb, vb, ob, isem, osem):
        ins = ((q_hbm, qb), (k_hbm, kb), (v_hbm, vb))

        def rd(x, t):
            slot = t % nbuf
            return pltpu.make_async_copy(ins[x][0].at[pl.ds(t * gs, gs)],
                                         ins[x][1].at[slot], isem.at[x, slot])

        def wr(t):
            return pltpu.make_async_copy(ob.at[t], o_hbm.at[pl.ds(t * gs, gs)],
                                         osem.at[t])

        def start_reads(t):
            for x in range(3):
                rd(x, t).start()

        for t in range(la):
            start_reads(t)

        def body(t, _):
            @pl.when(t + la < T)
            def _():
                start_reads(t + la)

            for x in range(3):
                rd(x, t).wait()
            slot = t % nbuf
            for g in range(gs):
                ob[t, g] = _attention_head(
                    qb[slot, g], kb[slot, g], vb[slot, g], c).astype(ob.dtype)

            @pl.when(t == T - w_early)
            def _():
                jax.lax.fori_loop(0, T - w_early, lambda i, _: wr(i).start(), None)

            @pl.when(t >= T - w_early)
            def _():
                wr(t).start()

        jax.lax.fori_loop(0, T, body, None)
        jax.lax.fori_loop(0, T, lambda i, _: wr(i).wait(), None)

    out = pl.pallas_call(
        kernel_function,
        grid=(),
        in_specs=[pl.BlockSpec(memory_space=pl.ANY)] * 3,
        out_specs=pl.BlockSpec(memory_space=pl.ANY),
        out_shape=jax.ShapeDtypeStruct((NH, Sq, D), q.dtype),
        scratch_shapes=[
            pltpu.VMEM((nbuf, gs, Sq, D), q.dtype),
            pltpu.VMEM((nbuf, gs, Sk, D), k.dtype),
            pltpu.VMEM((nbuf, gs, Sk, D), v.dtype),
            pltpu.VMEM((T, gs, Sq, D), q.dtype),
            pltpu.SemaphoreType.DMA((3, nbuf)),
            pltpu.SemaphoreType.DMA((T,)),
        ],
        compiler_params=pltpu.CompilerParams(vmem_limit_bytes=110 * 2**20),
    )(q.reshape(NH, Sq, D), k.reshape(NH, Sk, D), v.reshape(NH, Sk, D))
    return out.reshape(B, H, Sq, D)
```

```python
import math

import jax
import jax.numpy as jnp
import jax.experimental.pallas as pl
import jax.experimental.pallas.tpu as pltpu

HEADS_PER_CHUNK = 8
LOOKAHEAD = 3
WRITE_STREAMS = 32
WRITE_SETS = 2
SUBLANE_TILE = 16


def _attention_head(q, k, v, c):
    s = jax.lax.dot_general(q, k, (((1,), (1,)), ((), ())),
                            preferred_element_type=jnp.float32)
    m = jnp.max(s, axis=-1, keepdims=True)
    e = jnp.exp2((s - m) * c)
    l = jnp.sum(e, axis=-1, keepdims=True)
    o = jnp.dot(e.astype(v.dtype), v, preferred_element_type=jnp.float32)
    return o * (1.0 / l)


@jax.jit
def pallas_standalone__mha_softmax__near_ridge_kernel(
    q: jax.Array,
    k: jax.Array,
    v: jax.Array,
):
    B, H, Sq, D = q.shape
    Sk = k.shape[2]
    NH = B * H
    gs = math.gcd(HEADS_PER_CHUNK, NH)
    T = NH // gs
    la = min(LOOKAHEAD, T)
    nbuf = la + 1
    rows = gs * Sq
    nst = math.gcd(WRITE_STREAMS, rows // SUBLANE_TILE)
    rpart = rows // nst
    nset = math.gcd(WRITE_SETS, T)
    wg = T // nset
    c = math.log2(math.e) * (D ** -0.5)

    def kernel_function(q_hbm, k_hbm, v_hbm, o_hbm, qb, kb, vb, ob, isem, osem):
        ins = ((q_hbm, qb), (k_hbm, kb), (v_hbm, vb))

        def rd(x, t):
            slot = t % nbuf
            return pltpu.make_async_copy(ins[x][0].at[pl.ds(t * gs, gs)],
                                         ins[x][1].at[slot], isem.at[x, slot])

        def wr(s, p):
            idx = (pl.ds(s * wg, wg), pl.ds(p * rpart, rpart))
            return pltpu.make_async_copy(ob.at[idx], o_hbm.at[idx], osem.at[p])

        def start_reads(t):
            for x in range(3):
                rd(x, t).start()

        def compute(t):
            slot = t % nbuf
            for g in range(gs):
                ob[t, pl.ds(g * Sq, Sq), :] = _attention_head(
                    qb[slot, g], kb[slot, g], vb[slot, g], c).astype(ob.dtype)

        for t in range(la):
            start_reads(t)

        def body(t, _):
            @pl.when(t + la < T)
            def _():
                start_reads(t + la)

            for x in range(3):
                rd(x, t).wait()
            compute(t)

        jax.lax.fori_loop(0, T - 1, body, None)

        rd(0, T - 1).wait()
        if nset > 1:
            for p in range(nst):
                wr(0, p).start()
        rd(1, T - 1).wait()
        rd(2, T - 1).wait()
        compute(T - 1)
        if nset == 1:
            for p in range(nst):
                wr(0, p).start()

        for s in range(1, nset):
            for p in range(nst):
                wr(s - 1, p).wait()
                wr(s, p).start()
        for p in range(nst):
            wr(nset - 1, p).wait()

    out = pl.pallas_call(
        kernel_function,
        grid=(),
        in_specs=[pl.BlockSpec(memory_space=pl.ANY)] * 3,
        out_specs=pl.BlockSpec(memory_space=pl.ANY),
        out_shape=jax.ShapeDtypeStruct((T, rows, D), q.dtype),
        scratch_shapes=[
            pltpu.VMEM((nbuf, gs, Sq, D), q.dtype),
            pltpu.VMEM((nbuf, gs, Sk, D), k.dtype),
            pltpu.VMEM((nbuf, gs, Sk, D), v.dtype),
            pltpu.VMEM((T, rows, D), q.dtype),
            pltpu.SemaphoreType.DMA((3, nbuf)),
            pltpu.SemaphoreType.DMA((nst,)),
        ],
        compiler_params=pltpu.CompilerParams(vmem_limit_bytes=100 * 2**20),
    )(q.reshape(NH, Sq, D), k.reshape(NH, Sk, D), v.reshape(NH, Sk, D))
    return out.reshape(B, H, Sq, D)
```

```python
import math

import jax
import jax.numpy as jnp
import jax.experimental.pallas as pl
import jax.experimental.pallas.tpu as pltpu

UNROLL = 8
RING = 4
LOOKAHEAD = RING - 1
READ_PRIORITY = (1, 0, 1)
WRITE_PRIORITY = 1
WRITE_STREAMS = 32
WRITE_SETS = 2
HANDOFF = 3
SUBLANE_TILE = 16


def _attention_head(q, k, v, c):
    s = jax.lax.dot_general(q, k, (((1,), (1,)), ((), ())),
                            preferred_element_type=jnp.float32)
    m = jnp.max(s, axis=-1, keepdims=True)
    e = jnp.exp2((s - m) * c)
    l = jnp.sum(e, axis=-1, keepdims=True)
    o = jnp.dot(e.astype(v.dtype), v, preferred_element_type=jnp.float32)
    return o * (1.0 / l)


@jax.jit
def pallas_standalone__mha_softmax__near_ridge_kernel(
    q: jax.Array,
    k: jax.Array,
    v: jax.Array,
):
    B, H, Sq, D = q.shape
    Sk = k.shape[2]
    NH = B * H
    assert NH % UNROLL == 0 and NH >= 2 * UNROLL, "heads must fill >= 2 windows"
    T = NH // UNROLL
    rows = UNROLL * Sq
    nst = math.gcd(WRITE_STREAMS, rows // SUBLANE_TILE)
    rpart = rows // nst
    nset = WRITE_SETS if T % WRITE_SETS == 0 else T
    wg = T // nset
    assert wg <= T - 1
    c = math.log2(math.e) * (D ** -0.5)

    def kernel_function(q_hbm, k_hbm, v_hbm, o_hbm, qb, kb, vb, ob, isem, osem):
        ins = ((q_hbm, qb), (k_hbm, kb), (v_hbm, vb))

        def rd(x, n, slot):
            return pltpu.make_async_copy(ins[x][0].at[n], ins[x][1].at[slot],
                                         isem.at[x, slot])

        def wr(s, p):
            idx = (pl.ds(s * wg, wg), pl.ds(p * rpart, rpart))
            return pltpu.make_async_copy(ob.at[idx], o_hbm.at[idx], osem.at[p])

        def start_reads(n, slot):
            for x in range(3):
                rd(x, n, slot).start(priority=READ_PRIORITY[x])

        for n in range(LOOKAHEAD):
            start_reads(n, n)

        def body(i, _):
            for j in range(UNROLL):
                n = i * UNROLL + j
                slot, ahead = j % RING, (j + LOOKAHEAD) % RING
                if j + LOOKAHEAD < UNROLL:
                    start_reads(n + LOOKAHEAD, ahead)
                else:
                    @pl.when(i < T - 1)
                    def _():
                        start_reads(n + LOOKAHEAD, ahead)

                if j == UNROLL - HANDOFF:
                    @pl.when(i == T - 1)
                    def _():
                        for p in range(nst):
                            wr(0, p).start(priority=WRITE_PRIORITY)

                for x in range(3):
                    rd(x, n, slot).wait()
                ob[i, pl.ds(j * Sq, Sq), :] = _attention_head(
                    qb[slot], kb[slot], vb[slot], c).astype(ob.dtype)

        jax.lax.fori_loop(0, T, body, None)

        for s in range(1, nset):
            for p in range(nst):
                wr(s - 1, p).wait()
                wr(s, p).start(priority=WRITE_PRIORITY)
        for p in range(nst):
            wr(nset - 1, p).wait()

    out = pl.pallas_call(
        kernel_function,
        grid=(),
        in_specs=[pl.BlockSpec(memory_space=pl.ANY)] * 3,
        out_specs=pl.BlockSpec(memory_space=pl.ANY),
        out_shape=jax.ShapeDtypeStruct((T, rows, D), q.dtype),
        scratch_shapes=[
            pltpu.VMEM((RING, Sq, D), q.dtype),
            pltpu.VMEM((RING, Sk, D), k.dtype),
            pltpu.VMEM((RING, Sk, D), v.dtype),
            pltpu.VMEM((T, rows, D), q.dtype),
            pltpu.SemaphoreType.DMA((3, RING)),
            pltpu.SemaphoreType.DMA((nst,)),
        ],
        compiler_params=pltpu.CompilerParams(vmem_limit_bytes=64 * 2**20),
    )(q.reshape(NH, Sq, D), k.reshape(NH, Sk, D), v.reshape(NH, Sk, D))
    return out.reshape(B, H, Sq, D)
```

```python
import math

import jax
import jax.numpy as jnp
import numpy as np
import jax.experimental.pallas as pl
import jax.experimental.pallas.tpu as pltpu

UNROLL = 8
RING = 4
LOOKAHEAD = RING - 1
READ_PRIORITY = (1, 0, 1)
WRITE_PRIORITY = 1
WRITE_STREAMS = 32
WRITE_SETS = 2
HANDOFF = 3
SUBLANE_TILE = 16


def _round_to(x, dtype):
    return x.astype(dtype).astype(jnp.float32)


def _attention_head(q, k, v, scale):
    s = jax.lax.dot_general(q, k, (((1,), (1,)), ((), ())),
                            preferred_element_type=jnp.float32)
    s = _round_to(s, q.dtype)
    c = math.log2(math.e)
    if math.frexp(scale)[0] == 0.5:
        c *= scale
    else:
        s = _round_to(s * scale, q.dtype)
    m = jnp.max(s, axis=-1, keepdims=True)
    e = jnp.exp2((s - m) * c)
    l = jnp.sum(e, axis=-1, keepdims=True)
    o = jnp.dot(e.astype(v.dtype), v, preferred_element_type=jnp.float32)
    return o * (1.0 / l)


@jax.jit
def pallas_standalone__mha_softmax__near_ridge_kernel(
    q: jax.Array,
    k: jax.Array,
    v: jax.Array,
):
    B, H, Sq, D = q.shape
    Sk = k.shape[2]
    NH = B * H
    assert NH % UNROLL == 0 and NH >= 2 * UNROLL, "heads must fill >= 2 windows"
    T = NH // UNROLL
    rows = UNROLL * Sq
    nst = math.gcd(WRITE_STREAMS, rows // SUBLANE_TILE)
    rpart = rows // nst
    nset = WRITE_SETS if T % WRITE_SETS == 0 else T
    wg = T // nset
    assert wg <= T - 1
    scale = float(np.asarray(D ** -0.5).astype(q.dtype))

    def kernel_function(q_hbm, k_hbm, v_hbm, o_hbm, qb, kb, vb, ob, isem, osem):
        ins = ((q_hbm, qb), (k_hbm, kb), (v_hbm, vb))

        def rd(x, n, slot):
            return pltpu.make_async_copy(ins[x][0].at[n], ins[x][1].at[slot],
                                         isem.at[x, slot])

        def wr(s, p):
            idx = (pl.ds(s * wg, wg), pl.ds(p * rpart, rpart))
            return pltpu.make_async_copy(ob.at[idx], o_hbm.at[idx], osem.at[p])

        def start_reads(n, slot):
            for x in range(3):
                rd(x, n, slot).start(priority=READ_PRIORITY[x])

        for n in range(LOOKAHEAD):
            start_reads(n, n)

        def body(i, _):
            for j in range(UNROLL):
                n = i * UNROLL + j
                slot, ahead = j % RING, (j + LOOKAHEAD) % RING
                if j + LOOKAHEAD < UNROLL:
                    start_reads(n + LOOKAHEAD, ahead)
                else:
                    @pl.when(i < T - 1)
                    def _():
                        start_reads(n + LOOKAHEAD, ahead)

                if j == UNROLL - HANDOFF:
                    @pl.when(i == T - 1)
                    def _():
                        for p in range(nst):
                            wr(0, p).start(priority=WRITE_PRIORITY)

                for x in range(3):
                    rd(x, n, slot).wait()
                ob[i, pl.ds(j * Sq, Sq), :] = _attention_head(
                    qb[slot], kb[slot], vb[slot], scale).astype(ob.dtype)

        jax.lax.fori_loop(0, T, body, None)

        for s in range(1, nset):
            for p in range(nst):
                wr(s - 1, p).wait()
                wr(s, p).start(priority=WRITE_PRIORITY)
        for p in range(nst):
            wr(nset - 1, p).wait()

    out = pl.pallas_call(
        kernel_function,
        grid=(),
        in_specs=[pl.BlockSpec(memory_space=pl.ANY)] * 3,
        out_specs=pl.BlockSpec(memory_space=pl.ANY),
        out_shape=jax.ShapeDtypeStruct((T, rows, D), q.dtype),
        scratch_shapes=[
            pltpu.VMEM((RING, Sq, D), q.dtype),
            pltpu.VMEM((RING, Sk, D), k.dtype),
            pltpu.VMEM((RING, Sk, D), v.dtype),
            pltpu.VMEM((T, rows, D), q.dtype),
            pltpu.SemaphoreType.DMA((3, RING)),
            pltpu.SemaphoreType.DMA((nst,)),
        ],
        compiler_params=pltpu.CompilerParams(vmem_limit_bytes=64 * 2**20),
    )(q.reshape(NH, Sq, D), k.reshape(NH, Sk, D), v.reshape(NH, Sk, D))
    return out.reshape(B, H, Sq, D)
```
